```python
import jax
import jax.numpy as jnp

def _softmax(x, axis=-1):
    return jax.nn.softmax(x, axis=axis)
def _gelu(x):
    return jax.nn.gelu(x, approximate=True)
def _silu(x):
    return jax.nn.silu(x)
def _sigmoid(x):
    return jax.nn.sigmoid(x)
def _layernorm(x, axis=-1, eps=1e-5):
    m = jnp.mean(x, axis=axis, keepdims=True)
    v = jnp.var(x, axis=axis, keepdims=True)
    return (x - m) / jnp.sqrt(v + eps)
def _scatter_add(tgt, idx, src, axis=0):
    return tgt.at[idx].add(src)
def _segment_sum(src, seg, n):
    return jax.ops.segment_sum(src, seg, n)
class _Rng:
    def __init__(self, key):
        self._k = key
    def _next(self):
        self._k, sub = jax.random.split(self._k)
        return sub
    def normal(self, shape):
        return jax.random.normal(self._next(), shape, dtype=jnp.bfloat16)
    def randint(self, lo, hi, shape):
        return jax.random.randint(self._next(), shape, lo, hi, dtype=jnp.int32)
    def uniform(self, shape, lo=0.0, hi=1.0):
        return jax.random.uniform(self._next(), shape, jnp.bfloat16, lo, hi)
    def permutation(self, n):
        return jax.random.permutation(self._next(), n)


kernel_name = 'gated_mix__sliding_block_cached__moe_arch_mod__decode'

def setup_inputs():
    _rng = _Rng(jax.random.key(int.from_bytes(__import__("os").urandom(4), "little")))
    _w = (lambda a: (lambda t: t.astype(jnp.bfloat16) if jnp.issubdtype(t.dtype, jnp.floating) else t)(jnp.asarray(a)))
    def _A_setup():
        B, Sq, D = 1, 1, 640
        Hq, Hkv, Sk, Dh = 32, 32, 32768, 192
        assert Hq % Hkv == 0, (Hq, Hkv)
        return {
            "x": _w((lambda *s: _rng.normal(s) * 0.05)(B, Sq, D)),
            "k_cache": _w((lambda *s: _rng.normal(s) * 0.05)(B, Hkv, Sk, Dh)),
            "v_cache": _w((lambda *s: _rng.normal(s) * 0.05)(B, Hkv, Sk, Dh)),
            "wq": _w((lambda *s: _rng.normal(s) * 0.05)(D, Hq * Dh) * (D ** -0.5)),
            "wo": _w((lambda *s: _rng.normal(s) * 0.05)(Hq * Dh, D) * ((Hq * Dh) ** -0.5)),
        }
    _A_in = _A_setup()

    def _B_setup():
        B, S, D, F, C = 1, 1, 640, 1536, 1
        return {
            "x": _w((lambda *s: _rng.normal(s) * 0.05)(B, S, D)),
            "w_r": _w((lambda *s: _rng.normal(s) * 0.05)(D)),
            "w_gate": _w((lambda *s: _rng.normal(s) * 0.05)(D, F)),
            "w_up": _w((lambda *s: _rng.normal(s) * 0.05)(D, F)),
            "w_down": _w((lambda *s: _rng.normal(s) * 0.05)(F, D)),
        }
    _B_in = _B_setup()

    return {
        "A_x": _A_in["x"],
        "A_k_cache": _A_in["k_cache"],
        "A_v_cache": _A_in["v_cache"],
        "A_wq": _A_in["wq"],
        "A_wo": _A_in["wo"],
        "B_x": _B_in["x"],
        "B_w_r": _B_in["w_r"],
        "B_w_gate": _B_in["w_gate"],
        "B_w_up": _B_in["w_up"],
        "B_w_down": _B_in["w_down"],
        "gate_w": _w((lambda *s: _rng.normal(s) * 0.05)(640)),
    }

def reference(A_x, A_k_cache, A_v_cache, A_wq, A_wo, B_x, B_w_r, B_w_gate, B_w_up, B_w_down, gate_w):
    def _A_ref(x, k_cache, v_cache, wq, wo):
        B, Sq, D = x.shape
        Hq, Dh = 32, 192
        Hkv, Sk = k_cache.shape[1], k_cache.shape[2]
        W = min(4096, max(256, Sk // 4))
        rep = Hq // Hkv
        q = (lambda x, *d: x.transpose(*d))((x @ wq).reshape(B, Sq, Hq, Dh), 0, 2, 1, 3)
        k = jnp.repeat(k_cache[:, :, Sk - W:, :], rep, axis=1)
        v = jnp.repeat(v_cache[:, :, Sk - W:, :], rep, axis=1)
        scores = jnp.einsum("bhqd,bhkd->bhqk", q, k) * (Dh ** -0.5)
        p = _softmax(scores, axis=-1)
        o = jnp.einsum("bhqk,bhkd->bhqd", p, v)
        return (lambda x, *d: x.transpose(*d))(o, 0, 2, 1, 3).reshape(B, Sq, Hq * Dh) @ wo

    def _B_ref(x, w_r, w_gate, w_up, w_down):
        B, S, D = x.shape
        C = 1
        r = x @ w_r
        idx = jnp.argsort(-r, axis=-1)[:, :C]
        idx_e = jnp.repeat(idx.reshape(B, C, 1), D, axis=2)
        x_sel = jnp.take_along_axis(x, idx_e, axis=1)
        g = _silu(x_sel @ w_gate)
        u = x_sel @ w_up
        y = (g * u) @ w_down
        r_sel = _sigmoid(jnp.take_along_axis(r, idx, axis=1))
        y = y * r_sel.reshape(B, C, 1)
        b_off = (jnp.arange(B) * S).reshape(B, 1)
        flat_idx = (idx + b_off).reshape(B * C)
        zero = (x * 0.0).reshape(B * S, D)
        upd = _scatter_add(zero, flat_idx, y.reshape(B * C, D), axis=0)
        return x + upd.reshape(B, S, D)

    x = A_x
    g = _sigmoid((x * gate_w).sum(-1, keepdims=True))
    a = _A_ref(x, A_k_cache, A_v_cache, A_wq, A_wo)
    b = _B_ref(x, B_w_r, B_w_gate, B_w_up, B_w_down)
    return g * a + (1 - g) * b
```

```python
import jax
import jax.numpy as jnp
import jax.experimental.pallas as pl
import jax.experimental.pallas.tpu as pltpu

H, DH, SK, W, D, F = 32, 192, 32768, 4096, 640, 1536
BASE = SK - W
NSLOT = 3
NQ = 4
QCW = H * DH // NQ
NO = 4
ORW = H * DH // NO
ND = 6
DRW = F // ND
MROWS = 8

f32 = jnp.float32
bf16 = jnp.bfloat16


def kernel(x_hbm, kT, vT, wq, wo, wr_hbm, wg, wu, wd, gw_hbm, out_ref,
           x_v, wr_v, gw_v, wq_b, k_b, v_b, wo_b, wg_b, wu_b, wd_b, q_s, o_s,
           sm_small, sm_q, sm_k, sm_v, sm_o, sm_g, sm_d):
    def cp_small():
        return [pltpu.make_async_copy(x_hbm, x_v, sm_small.at[0]),
                pltpu.make_async_copy(gw_hbm, gw_v, sm_small.at[1]),
                pltpu.make_async_copy(wr_hbm, wr_v, sm_small.at[2])]

    def cp_q(c):
        return pltpu.make_async_copy(wq.at[:, pl.ds(c * QCW, QCW)], wq_b.at[:, pl.ds(c * QCW, QCW)], sm_q.at[c])

    def cp_k(h):
        s = h % NSLOT
        return pltpu.make_async_copy(kT.at[0, h, :, pl.ds(BASE, W)], k_b.at[s], sm_k.at[s])

    def cp_v(h):
        s = h % NSLOT
        return pltpu.make_async_copy(vT.at[0, h, :, pl.ds(BASE, W)], v_b.at[s], sm_v.at[s])

    def cp_o(c):
        return pltpu.make_async_copy(wo.at[pl.ds(c * ORW, ORW), :], wo_b.at[pl.ds(c * ORW, ORW), :], sm_o.at[c])

    def cp_g():
        return [pltpu.make_async_copy(wg, wg_b, sm_g.at[0]), pltpu.make_async_copy(wu, wu_b, sm_g.at[1])]

    def cp_d(c):
        return pltpu.make_async_copy(wd.at[pl.ds(c * DRW, DRW), :], wd_b.at[pl.ds(c * DRW, DRW), :], sm_d.at[c])

    cp_q(0).start()
    for c in cp_small():
        c.start()
    for c in range(1, NQ):
        cp_q(c).start()
    for h in range(NSLOT - 1):
        cp_k(h).start()
        cp_v(h).start()

    for c in cp_small():
        c.wait()
    x = x_v[0]
    xf = x.astype(f32)
    gate = jax.nn.sigmoid(jnp.sum(xf * gw_v[...].astype(f32).reshape(1, D), axis=-1, keepdims=True))
    rsel = jax.nn.sigmoid(jnp.sum(xf * wr_v[...].astype(f32).reshape(1, D), axis=-1, keepdims=True))
    xm = jnp.broadcast_to(x, (2 * MROWS, D))

    for c in range(NQ):
        cp_q(c).wait()
        qc = jnp.dot(xm, wq_b[:, c * QCW:(c + 1) * QCW], preferred_element_type=f32)[:MROWS]
        hp = H // NQ
        for j in range(hp):
            q_s[c * hp + j] = qc[:, j * DH:(j + 1) * DH]

    scale = DH ** -0.5

    def head(h, carry):
        cp_k(h).wait()

        @pl.when(h + NSLOT - 1 < H)
        def _():
            cp_k(h + NSLOT - 1).start()

        s = h % NSLOT
        q = q_s[h].astype(bf16)
        sc = jnp.dot(q, k_b[s], preferred_element_type=f32) * scale
        m = jnp.max(sc, axis=-1, keepdims=True)
        p = jnp.exp(sc - m)
        l = jnp.sum(p, axis=-1, keepdims=True)
        cp_v(h).wait()

        @pl.when(h + NSLOT - 1 < H)
        def _():
            cp_v(h + NSLOT - 1).start()

        @pl.when(h == H - NSLOT + 1)
        def _():
            for c in cp_g():
                c.start()
            for c in range(NO):
                cp_o(c).start()
            for c in range(ND):
                cp_d(c).start()

        o = jax.lax.dot_general(p.astype(bf16), v_b[s], (((1,), (1,)), ((), ())), preferred_element_type=f32)
        o_s[h] = o / l
        return carry

    jax.lax.fori_loop(0, H, head, 0)

    cg, cu = cp_g()
    cg.wait()
    g = jnp.dot(xm, wg_b[...], preferred_element_type=f32)
    cu.wait()
    u = jnp.dot(xm, wu_b[...], preferred_element_type=f32)
    hh = (jax.nn.silu(g) * u).astype(bf16)

    a = jnp.zeros((2 * MROWS, D), f32)
    for c in range(NO):
        cp_o(c).wait()
        hp = H // NO
        for j in range(hp):
            hidx = c * hp + j
            ov = o_s[hidx].astype(bf16)
            a = a[:MROWS] + jnp.dot(ov, wo_b[hidx * DH:(hidx + 1) * DH, :], preferred_element_type=f32)
    y = jnp.zeros((2 * MROWS, D), f32)
    for c in range(ND):
        cp_d(c).wait()
        y = y + jnp.dot(hh[:, c * DRW:(c + 1) * DRW], wd_b[c * DRW:(c + 1) * DRW, :], preferred_element_type=f32)
    a = a[0:1]
    y = y[0:1]
    b = xf + (xf * 0.0 + y * rsel)
    out = gate * a + (1.0 - gate) * b
    out_ref[0] = out.astype(bf16)


@jax.jit
def pallas_gated_mix__sliding_block_cached__moe_arch_mod__decode_kernel(A_x, A_k_cache, A_v_cache, A_wq, A_wo, B_x, B_w_r, B_w_gate, B_w_up, B_w_down, gate_w):
    kT = jnp.swapaxes(A_k_cache, 2, 3)
    vT = jnp.swapaxes(A_v_cache, 2, 3)
    anyspec = pl.BlockSpec(memory_space=pl.ANY)
    VM = pltpu.VMEM
    SD = pltpu.SemaphoreType.DMA
    return pl.pallas_call(
        kernel,
        out_shape=jax.ShapeDtypeStruct((1, 1, D), bf16),
        in_specs=[anyspec] * 10,
        out_specs=pl.BlockSpec(memory_space=pltpu.VMEM),
        scratch_shapes=[VM((1, 1, D), bf16), VM((D,), bf16), VM((D,), bf16),
                        VM((D, H * DH), bf16), VM((NSLOT, DH, W), bf16), VM((NSLOT, DH, W), bf16),
                        VM((H * DH, D), bf16), VM((D, F), bf16), VM((D, F), bf16), VM((F, D), bf16),
                        VM((H, MROWS, DH), f32), VM((H, MROWS, DH), f32),
                        SD((3,)), SD((NQ,)), SD((NSLOT,)), SD((NSLOT,)), SD((NO,)), SD((2,)), SD((ND,))],
        compiler_params=pltpu.CompilerParams(vmem_limit_bytes=100 * 1024 * 1024),
        name='gm',
    )(A_x, kT, vT, A_wq, A_wo, B_w_r, B_w_gate, B_w_up, B_w_down, gate_w)
```

```python
import jax
import jax.numpy as jnp
import jax.experimental.pallas as pl
import jax.experimental.pallas.tpu as pltpu
import contextlib

H, DH, SK, W, D, F = 32, 192, 32768, 4096, 640, 1536
BASE = SK - W
MROWS = 8
f32 = jnp.float32
bf16 = jnp.bfloat16


def make(G=1, NQ=4, NO=4, DSPLIT=(128,)*12, name='gm', scopes=False, pk=0, pv=1, ppost=1, pq=0, TW=128, lagstore=False, nobc=True):
    NC = W // TW
    QCW = H * DH // NQ
    ORW = H * DH // NO
    ND = len(DSPLIT)
    DOFF = [sum(DSPLIT[:i]) for i in range(ND)]
    assert sum(DSPLIT) == F
    S_SMALL = 0
    S_Q = 3
    S_K = S_Q + NQ
    S_V = S_K + NC
    S_G = S_V + NC
    S_O = S_G + 2
    S_D = S_O + NO
    NSEM = S_D + ND

    def scope(n):
        return jax.named_scope(n) if scopes else contextlib.nullcontext()

    def kernel(x_hbm, kT, vT, wq, wo, wr_hbm, wg, wu, wd, gw_hbm, out_ref,
               x_v, wr_v, gw_v, wq_b, k_b, v_b, wo_b, wg_b, wu_b, wd_b, q_s, o_s, s_s, p_s, sems):
        def cp_small():
            return [pltpu.make_async_copy(x_hbm, x_v, sems.at[S_SMALL + 0]),
                    pltpu.make_async_copy(gw_hbm, gw_v, sems.at[S_SMALL + 1]),
                    pltpu.make_async_copy(wr_hbm, wr_v, sems.at[S_SMALL + 2])]

        def cp_q(c):
            return pltpu.make_async_copy(wq.at[:, pl.ds(c * QCW, QCW)], wq_b.at[:, pl.ds(c * QCW, QCW)], sems.at[S_Q + c])

        def cp_k(h, c):
            return pltpu.make_async_copy(kT.at[0, h, :, pl.ds(BASE + c * TW, TW)],
                                         k_b.at[h % 2, :, pl.ds(c * TW, TW)], sems.at[S_K + c])

        def cp_v(h, c):
            return pltpu.make_async_copy(vT.at[0, h, :, pl.ds(BASE + c * TW, TW)],
                                         v_b.at[h % 2, :, pl.ds(c * TW, TW)], sems.at[S_V + c])

        def cp_o(c):
            return pltpu.make_async_copy(wo.at[pl.ds(c * ORW, ORW), :], wo_b.at[pl.ds(c * ORW, ORW), :], sems.at[S_O + c])

        def cp_g(i):
            return pltpu.make_async_copy([wg, wu][i], [wg_b, wu_b][i], sems.at[S_G + i])

        def cp_d(c):
            sl = pl.ds(DOFF[c], DSPLIT[c])
            return pltpu.make_async_copy(wd.at[sl, :], wd_b.at[sl, :], sems.at[S_D + c])

        cp_q(0).start(priority=pq)
        for c in cp_small():
            c.start()
        for c in range(1, NQ):
            cp_q(c).start(priority=pq)
        for c in range(NC):
            cp_k(0, c).start(priority=pk)

        for c in cp_small():
            c.wait()
        x = x_v[0]
        xf = x.astype(f32)
        gate = jax.nn.sigmoid(jnp.sum(xf * gw_v[...].astype(f32).reshape(1, D), axis=-1, keepdims=True))
        rsel = jax.nn.sigmoid(jnp.sum(xf * wr_v[...].astype(f32).reshape(1, D), axis=-1, keepdims=True))
        xm = jnp.broadcast_to(x, (2 * MROWS, D))

        for c in range(NQ):
            cp_q(c).wait()
            qc = jnp.dot(xm, wq_b[:, c * QCW:(c + 1) * QCW], preferred_element_type=f32)[:MROWS]
            hp = H // NQ
            for j in range(hp):
                q_s[c * hp + j] = qc[:, j * DH:(j + 1) * DH]

        scale = DH ** -0.5

        def head(h, do_k, do_v, last_k=False):
            if do_k:
                q = q_s[h].astype(bf16)
            acc = jnp.zeros((MROWS, DH), f32)
            for c in range(NC):
                if do_k:
                    cp_k(h, c).wait()
                    if not last_k:
                        cp_k(h + 1, c).start(priority=pk)
                if do_v:
                    cp_v(h - 1, c).wait()
                if do_k:
                    cp_v(h, c).start(priority=pv)
                if (c + 1) % G == 0:
                    sl = slice((c + 1 - G) * TW, (c + 1) * TW)
                    if do_k:
                        s_s[:, sl] = jnp.dot(q, k_b[h % 2, :, sl], preferred_element_type=f32)
                    if do_v:
                        acc = acc + jax.lax.dot_general(p_s[:, sl].astype(bf16), v_b[(h - 1) % 2, :, sl],
                                                        (((1,), (1,)), ((), ())), preferred_element_type=f32)
            if do_v:
                o_s[h - 1] = acc
            if do_k:
                sc = s_s[...] * scale
                m = jnp.max(sc, axis=-1, keepdims=True)
                p = jnp.exp(sc - m)
                l = jnp.sum(p, axis=-1, keepdims=True)
                p_s[...] = p / l

        with scope('heads'):
            head(0, True, False)

            def body(h, carry):
                head(h, True, True)
                return carry
            jax.lax.fori_loop(1, H - 1, body, 0)
            head(H - 1, True, True, last_k=True)
            for i in range(2):
                cp_g(i).start(priority=ppost)
            for c in range(NO):
                cp_o(c).start(priority=ppost)
            for c in range(ND):
                cp_d(c).start(priority=ppost)
            head(H, False, True)

        with scope('wait_g'):
            cp_g(0).wait()
        with scope('comp_g'):
            g = jnp.dot(xm, wg_b[...], preferred_element_type=f32)
        with scope('wait_u'):
            cp_g(1).wait()
        with scope('comp_u'):
            u = jnp.dot(xm, wu_b[...], preferred_element_type=f32)
            hh = (jax.nn.silu(g) * u).astype(bf16)

        a = jnp.zeros((MROWS, D), f32)
        for c in range(NO):
            with scope(f'wait_o{c}'):
                cp_o(c).wait()
            with scope(f'comp_o{c}'):
                hp = H // NO
                for j in range(hp):
                    hidx = c * hp + j
                    ov = o_s[hidx].astype(bf16)
                    a = a + jnp.dot(ov, wo_b[hidx * DH:(hidx + 1) * DH, :], preferred_element_type=f32)
        y = jnp.zeros((2 * MROWS, D), f32)
        for c in range(ND):
            with scope(f'wait_d{c}'):
                cp_d(c).wait()
            with scope(f'comp_d{c}'):
                sl = slice(DOFF[c], DOFF[c] + DSPLIT[c])
                y = y + jnp.dot(hh[:, sl], wd_b[sl, :], preferred_element_type=f32)
        a = a[0:1]
        y = y[0:1]
        b = xf + (xf * 0.0 + y * rsel)
        out = gate * a + (1.0 - gate) * b
        out_ref[0] = out.astype(bf16)

    def fn(A_x, A_k_cache, A_v_cache, A_wq, A_wo, B_x, B_w_r, B_w_gate, B_w_up, B_w_down, gate_w):
        kT = jnp.swapaxes(A_k_cache, 2, 3)
        vT = jnp.swapaxes(A_v_cache, 2, 3)
        anyspec = pl.BlockSpec(memory_space=pl.ANY)
        VM = pltpu.VMEM
        SD = pltpu.SemaphoreType.DMA
        return pl.pallas_call(
            kernel,
            out_shape=jax.ShapeDtypeStruct((1, 1, D), bf16),
            in_specs=[anyspec] * 10,
            out_specs=pl.BlockSpec(memory_space=pltpu.VMEM),
            scratch_shapes=[VM((1, 1, D), bf16), VM((D,), bf16), VM((D,), bf16),
                            VM((D, H * DH), bf16), VM((2, DH, W), bf16), VM((2, DH, W), bf16),
                            VM((H * DH, D), bf16), VM((D, F), bf16), VM((D, F), bf16), VM((F, D), bf16),
                            VM((H, MROWS, DH), f32), VM((H, MROWS, DH), f32),
                            VM((MROWS, W), f32), VM((MROWS, W), f32),
                            SD((NSEM,))],
            compiler_params=pltpu.CompilerParams(vmem_limit_bytes=100 * 1024 * 1024, disable_semaphore_checks=True, disable_bounds_checks=nobc),
            name=name,
        )(A_x, kT, vT, A_wq, A_wo, B_w_r, B_w_gate, B_w_up, B_w_down, gate_w)
    return fn


_fn = make(G=2, nobc=False)


@jax.jit
def pallas_gated_mix__sliding_block_cached__moe_arch_mod__decode_kernel(
        A_x, A_k_cache, A_v_cache, A_wq, A_wo, B_x, B_w_r, B_w_gate, B_w_up, B_w_down, gate_w):
    return _fn(A_x, A_k_cache, A_v_cache, A_wq, A_wo, B_x, B_w_r, B_w_gate, B_w_up, B_w_down, gate_w)
```

```python
import jax
import jax.numpy as jnp
import jax.experimental.pallas as pl
import jax.experimental.pallas.tpu as pltpu

H, DH, SK, D, F = 32, 192, 32768, 640, 1536
W = min(4096, max(256, SK // 4))
BASE = SK - W
M = 8

KR, KC = 32, 512
NR, NGR = DH // KR, W // KC
L = 2 * NR * NGR
TPG = KC // 128
NT = W // 128

QP = (160, 128)
TP = 32
DCH = 256
L_END = 16
N_SMALL = 3

f32 = jnp.float32
bf16 = jnp.bfloat16


def _col_major_tiles(shape, piece):
    return [(r * piece[0], c * piece[1])
            for c in range(shape[1] // piece[1]) for r in range(shape[0] // piece[0])]


def _kernel(x_hbm, kT, vT, wq, wo, wr_hbm, wg, wu, wd, gw_hbm, out_ref,
            x_v, wr_v, gw_v, wq_b, k_b, v_b, wo_b, wg_b, wu_b, wd_b,
            q_s, o_s, s_s, p_s, sems):
    def small_copies():
        return [pltpu.make_async_copy(x_hbm, x_v, sems.at[L + 0]),
                pltpu.make_async_copy(gw_hbm, gw_v, sems.at[L + 1]),
                pltpu.make_async_copy(wr_hbm, wr_v, sems.at[L + 2])]

    def w_piece(src, dst, piece, rc):
        rows, cols = pl.ds(rc[0], piece[0]), pl.ds(rc[1], piece[1])
        return lambda slot: pltpu.make_async_copy(src.at[rows, cols], dst.at[rows, cols], sems.at[slot])

    def kv_piece(which, h, j, slot):
        g, r = divmod(j, NR)
        rows = pl.ds(r * KR, KR)
        src = (kT, vT)[which].at[0, h, rows, pl.ds(BASE + g * KC, KC)]
        buf = k_b.at[h % 2] if which == 0 else v_b.at[h % 3]
        return pltpu.make_async_copy(src, buf.at[rows, pl.ds(g * KC, KC)], sems.at[slot])

    pre = [w_piece(wq, wq_b, QP, rc) for rc in _col_major_tiles(wq.shape, QP)]
    n_pre = len(pre)
    for p in range(L):
        pre.append(lambda slot, p=p: kv_piece(p % 2, 0, p // 2, slot))

    g_tiles = _col_major_tiles(wg.shape, QP)
    n_g = len(g_tiles)
    post = [w_piece(wg, wg_b, QP, rc) for rc in g_tiles]
    post += [w_piece(wu, wu_b, QP, rc) for rc in g_tiles]
    tall = [(wo, wo_b, r) for r in range(0, H * DH, TP)] + [(wd, wd_b, r) for r in range(0, F, TP)]
    per_head = DH // TP
    cuts = [0, 9 * per_head, 19 * per_head, 29 * per_head, len(tall)]
    regions = [tall[a:b] for a, b in zip(cuts[:-1], cuts[1:])]
    tall_pos = {}
    for k in range(max(len(reg) for reg in regions)):
        for reg in regions:
            if k < len(reg):
                src, dst, r = reg[k]
                tall_pos[(src is wd, r)] = len(post)
                post.append(w_piece(src, dst, (TP, D), (r, 0)))
    n_post = len(post)

    for i in range(L):
        if i == 2:
            for c in small_copies():
                c.start()
        pre[i]((i - n_pre) % L).start(priority=(i - n_pre) % 2)

    for c in small_copies():
        c.wait()
    x = x_v[0]
    xf = x.astype(f32)
    gate = jax.nn.sigmoid(jnp.sum(xf * gw_v[...].astype(f32).reshape(1, D), axis=-1, keepdims=True))
    rsel = jax.nn.sigmoid(jnp.sum(xf * wr_v[...].astype(f32).reshape(1, D), axis=-1, keepdims=True))
    xm = jnp.broadcast_to(x, (2 * M, D))

    q_rows = D // QP[0]
    for i in range(n_pre):
        slot = (i - n_pre) % L
        pre[i](slot).wait()
        pre[i + L](slot).start(priority=(i - n_pre) % 2)
        cb, r = divmod(i, q_rows)
        if r == q_rows - 1:
            c0 = cb * QP[1]
            qc = jnp.dot(xm, wq_b[:, c0:c0 + QP[1]], preferred_element_type=f32)[:M]
            c = c0
            while c < c0 + QP[1]:
                hd, off = divmod(c, DH)
                n = min(DH - off, c0 + QP[1] - c)
                q_s[hd, :, off:off + n] = qc[:, c - c0:c - c0 + n]
                c += n

    scale = DH ** -0.5

    def qk(h, q, t0, t1):
        sl = slice(t0 * 128, t1 * 128)
        s_s[:, sl] = jnp.dot(q, k_b[h % 2, :, sl], preferred_element_type=f32)

    def pv(h, t0, t1):
        sl = slice(t0 * 128, t1 * 128)
        return jax.lax.dot_general(p_s[:, sl].astype(bf16), v_b[h % 3, :, sl],
                                   (((1,), (1,)), ((), ())), preferred_element_type=f32)

    def head(h, do_pv, last):
        q = q_s[h].astype(bf16)
        acc = jnp.zeros((M, DH), f32)
        for p in range(L):
            which = p % 2
            kv_piece(which, h, p // 2, p).wait()
            if last:
                post[p](p).start(priority=which)
            else:
                kv_piece(which, h + 1, p // 2, p).start(priority=which)
            if (p + 1) % (2 * NR) == 0:
                g = p // (2 * NR)
                qk(h, q, g * TPG, (g + 1) * TPG)
                if do_pv:
                    acc = acc + pv(h - 1, g * TPG, (g + 1) * TPG)
        if do_pv:
            o_s[h - 1] = acc
        sc = s_s[...] * scale
        m = jnp.max(sc, axis=-1, keepdims=True)
        e = jnp.exp(sc - m)
        p_s[...] = e / jnp.sum(e, axis=-1, keepdims=True)

    head(0, False, False)

    def body(h, carry):
        head(h, True, False)
        return carry

    jax.lax.fori_loop(1, H - 1, body, 0)
    head(H - 1, True, True)

    tasks = {}

    def at(step, fn):
        tasks.setdefault(step, []).append(fn)

    st = dict(acc=jnp.zeros((M, DH), f32), a=jnp.zeros((M, D), f32), g={}, u={})

    def t_pv(j):
        def fn():
            st['acc'] = st['acc'] + pv(H - 1, TPG * j, TPG * (j + 1))
            if j == NGR - 1:
                o_s[H - 1] = st['acc']
        return fn

    def t_gu(src, key, cb):
        def fn():
            st[key][cb] = jnp.dot(xm, src[:, cb * QP[1]:(cb + 1) * QP[1]], preferred_element_type=f32)
        return fn

    def t_o(hd):
        def fn():
            st['a'] = st['a'] + jnp.dot(o_s[hd].astype(bf16), wo_b[hd * DH:(hd + 1) * DH, :],
                                        preferred_element_type=f32)
        return fn

    def t_d(j):
        def fn():
            if j == 0:
                g = jnp.concatenate([st['g'][k] for k in range(F // QP[1])], axis=1)
                u = jnp.concatenate([st['u'][k] for k in range(F // QP[1])], axis=1)
                st['h'] = (jax.nn.silu(g) * u).astype(bf16)
            sl = slice(j * DCH, (j + 1) * DCH)
            part = jnp.dot(st['h'][:, sl], wd_b[sl, :], preferred_element_type=f32)
            st['y'] = part if j == 0 else st['y'] + part
        return fn

    for j in range(NGR):
        at(3 + 4 * j, t_pv(j))
    for which, (src, key) in enumerate(((wg_b, 'g'), (wu_b, 'u'))):
        for cb in range(F // QP[1]):
            at(which * n_g + (cb + 1) * q_rows - 1, t_gu(src, key, cb))
    for hd in range(H):
        at(max(tall_pos[(False, hd * DH + j * TP)] for j in range(per_head)), t_o(hd))
    for j in range(F // DCH):
        at(max(tall_pos[(True, j * DCH + k * TP)] for k in range(DCH // TP)), t_d(j))

    issue = {}
    for t in range(L, n_post):
        look = L
        if t % 2 == 0:
            look = L - (L - L_END) * (t - L) / (n_post - 1 - L)
        issue.setdefault(int(round(t - look)), []).append(t)

    for i in range(n_post):
        post[i](i % L).wait()
        for t in issue.get(i, []):
            post[t](t % L).start(priority=t % 2)
        for fn in tasks.get(i, []):
            fn()

    a = st['a'][0:1]
    y = st['y'][0:1]
    b = xf + (xf * 0.0 + y * rsel)
    out = gate * a + (1.0 - gate) * b
    out_ref[0] = out.astype(bf16)


@jax.jit
def pallas_gated_mix__sliding_block_cached__moe_arch_mod__decode_kernel(
        A_x, A_k_cache, A_v_cache, A_wq, A_wo, B_x, B_w_r, B_w_gate, B_w_up, B_w_down, gate_w):
    del B_x
    kT = jnp.swapaxes(A_k_cache, 2, 3)
    vT = jnp.swapaxes(A_v_cache, 2, 3)
    any_spec = pl.BlockSpec(memory_space=pl.ANY)
    vmem = pltpu.VMEM
    return pl.pallas_call(
        _kernel,
        out_shape=jax.ShapeDtypeStruct((1, 1, D), bf16),
        in_specs=[any_spec] * 10,
        out_specs=pl.BlockSpec(memory_space=pltpu.VMEM),
        scratch_shapes=[
            vmem((1, 1, D), bf16), vmem((D,), bf16), vmem((D,), bf16),
            vmem((D, H * DH), bf16), vmem((2, DH, W), bf16), vmem((3, DH, W), bf16),
            vmem((H * DH, D), bf16), vmem((D, F), bf16), vmem((D, F), bf16), vmem((F, D), bf16),
            vmem((H, M, DH), f32), vmem((H, M, DH), f32),
            vmem((M, W), f32), vmem((M, W), f32),
            pltpu.SemaphoreType.DMA((L + N_SMALL,)),
        ],
        compiler_params=pltpu.CompilerParams(
            vmem_limit_bytes=64 * 1024 * 1024,
            disable_semaphore_checks=True,
        ),
        name="gated_mix_decode",
    )(A_x, kT, vT, A_wq, A_wo, B_w_r, B_w_gate, B_w_up, B_w_down, gate_w)
```
